```python
import os as _os
_os.environ.setdefault("JAX_PLATFORMS", "cpu")
import jax
import jax.numpy as jnp

def _softmax(x, axis=-1):
    return jax.nn.softmax(x, axis=axis)
def _gelu(x):
    return jax.nn.gelu(x, approximate=True)
def _silu(x):
    return jax.nn.silu(x)
def _sigmoid(x):
    return jax.nn.sigmoid(x)
def _layernorm(x, axis=-1, eps=1e-5):
    m = jnp.mean(x, axis=axis, keepdims=True)
    v = jnp.var(x, axis=axis, keepdims=True)
    return (x - m) / jnp.sqrt(v + eps)
def _scatter_add(tgt, idx, src, axis=0):
    return tgt.at[idx].add(src)
def _segment_sum(src, seg, n):
    return jax.ops.segment_sum(src, seg, n)
class _Rng:
    def __init__(self, key):
        self._k = key
    def _next(self):
        self._k, sub = jax.random.split(self._k)
        return sub
    def normal(self, shape):
        return jax.random.normal(self._next(), shape, dtype=jnp.bfloat16)
    def randint(self, lo, hi, shape):
        return jax.random.randint(self._next(), shape, lo, hi, dtype=jnp.int32)
    def uniform(self, shape, lo=0.0, hi=1.0):
        return jax.random.uniform(self._next(), shape, jnp.bfloat16, lo, hi)
    def permutation(self, n):
        return jax.random.permutation(self._next(), n)


kernel_name = 'standalone__gqa_block_cached__near_ridge'

def setup_inputs():
    _rng = _Rng(jax.random.key(int.from_bytes(__import__("os").urandom(4), "little")))
    _w = (lambda a: (lambda t: t.astype(jnp.bfloat16) if jnp.issubdtype(t.dtype, jnp.floating) else t)(jnp.asarray(a)))
    B, Sq, D = 8, 144, 448
    Hq, Hkv, Sk, Dh = 16, 8, 2048, 256
    assert Hq % Hkv == 0, (Hq, Hkv)
    return {
        "x": _w((lambda *s: _rng.normal(s) * 0.8)(B, Sq, D)),
        "k_cache": _w((lambda *s: _rng.normal(s) * 0.8)(B, Hkv, Sk, Dh)),
        "v_cache": _w((lambda *s: _rng.normal(s) * 0.05)(B, Hkv, Sk, Dh)),
        "wq": _w((lambda *s: _rng.normal(s) * 0.8)(D, Hq * Dh) * (D ** -0.5)),
        "wo": _w((lambda *s: _rng.normal(s) * 0.05)(Hq * Dh, D) * ((Hq * Dh) ** -0.5)),
    }

def reference(x, k_cache, v_cache, wq, wo):
    B, Sq, D = x.shape
    Hq, Dh = 16, 256
    Hkv = k_cache.shape[1]
    rep = Hq // Hkv
    q = (lambda x, *d: x.transpose(*d))((x @ wq).reshape(B, Sq, Hq, Dh), 0, 2, 1, 3)
    k = jnp.repeat(k_cache, rep, axis=1)
    v = jnp.repeat(v_cache, rep, axis=1)
    scores = jnp.einsum("bhqd,bhkd->bhqk", q, k) * (Dh ** -0.5)
    p = _softmax(scores, axis=-1)
    o = jnp.einsum("bhqk,bhkd->bhqd", p, v)
    return (lambda x, *d: x.transpose(*d))(o, 0, 2, 1, 3).reshape(B, Sq, Hq * Dh) @ wo
```

```python
import functools

import jax
import jax.numpy as jnp
import jax.experimental.pallas as pl
import jax.experimental.pallas.tpu as pltpu

_LOG2E = 1.4426950408889634
_NT = (((1,), (1,)), ((), ()))
_RC = 16


def _kernel(x_ref, k_ref, v_ref, wq_ref, wot_ref, o_ref, acc_ref, p_ref, *, dh, scale):
    h = pl.program_id(0)
    b = pl.program_id(1)
    never = h < 0
    sq = x_ref.shape[0]
    sk = k_ref.shape[0]
    qf = jnp.dot(x_ref[...], wq_ref[...], preferred_element_type=jnp.float32)
    q = (qf * (scale * _LOG2E)).astype(jnp.bfloat16)

    def qk(r):
        return jax.lax.dot_general(q[:, r * dh:(r + 1) * dh], k_ref[...], _NT,
                                   preferred_element_type=jnp.float32)

    def softmax(r, s):
        for c in range(sq // _RC):
            sc = s[c * _RC:(c + 1) * _RC, :]
            m = jnp.max(sc, axis=-1, keepdims=True)
            p_ref[r, c * _RC:(c + 1) * _RC, :] = jnp.exp2(sc - m).astype(jnp.bfloat16)

    def inv_rowsum(r, dep):
        p = p_ref[r].astype(jnp.float32)
        lp = p[:, 0:128]
        for t in range(1, sk // 128):
            lp = lp + p[:, t * 128:(t + 1) * 128]
        lp = jnp.where(never, dep, lp)
        return 1.0 / jnp.sum(lp, axis=-1, keepdims=True)

    def pv(r):
        return jnp.dot(p_ref[r], v_ref[...], preferred_element_type=jnp.float32)

    s0 = qk(0)
    softmax(0, s0)
    s1 = qk(1)
    o0 = pv(0)
    r0 = inv_rowsum(0, o0[:, :128])
    softmax(1, s1)
    o1 = pv(1)
    r1 = inv_rowsum(1, o1[:, :128])
    oc = jnp.concatenate(
        [(o0 * r0).astype(jnp.bfloat16), (o1 * r1).astype(jnp.bfloat16)], axis=1)
    y = jax.lax.dot_general(oc, wot_ref[...], _NT, preferred_element_type=jnp.float32)
    acc_ref[b] = jnp.where(h == 0, 0.0, acc_ref[b]) + y

    @pl.when(h == pl.num_programs(0) - 1)
    def _():
        o_ref[...] = acc_ref[b].astype(o_ref.dtype)


@jax.jit
def pallas_standalone__gqa_block_cached__near_ridge_kernel(
    x: jax.Array,
    k_cache: jax.Array,
    v_cache: jax.Array,
    wq: jax.Array,
    wo: jax.Array,
):
    B, Sq, D = x.shape
    _, Hkv, Sk, Dh = k_cache.shape
    rep = wq.shape[1] // Dh // Hkv
    assert rep == 2
    kern = functools.partial(_kernel, dh=Dh, scale=Dh ** -0.5)
    return pl.pallas_call(
        kern,
        grid=(Hkv, B),
        in_specs=[
            pl.BlockSpec((None, Sq, D), lambda h, b: (b, 0, 0)),
            pl.BlockSpec((None, None, Sk, Dh), lambda h, b: (b, h, 0, 0)),
            pl.BlockSpec((None, None, Sk, Dh), lambda h, b: (b, h, 0, 0)),
            pl.BlockSpec((D, rep * Dh), lambda h, b: (0, h)),
            pl.BlockSpec((D, rep * Dh), lambda h, b: (0, h)),
        ],
        out_specs=pl.BlockSpec(
            (None, Sq, D), lambda h, b: (jnp.where(h == Hkv - 1, b, 0), 0, 0)),
        out_shape=jax.ShapeDtypeStruct((B, Sq, D), x.dtype),
        scratch_shapes=[
            pltpu.VMEM((B, Sq, D), jnp.float32),
            pltpu.VMEM((rep, Sq, Sk), jnp.bfloat16),
        ],
        compiler_params=pltpu.CompilerParams(
            dimension_semantics=("arbitrary", "arbitrary"),
            vmem_limit_bytes=64 * 1024 * 1024,
        ),
    )(x, k_cache, v_cache, wq, wo.T)
```

```python
import functools

import jax
import jax.numpy as jnp
from jax import lax
import jax.experimental.pallas as pl
import jax.experimental.pallas.tpu as pltpu

_LOG2E = 1.4426950408889634
_NT = (((1,), (1,)), ((), ()))
_RC = 16
_U = 4
_NBLK = 2
_KG = 256
_G0 = 2
_P2T = 3


def _kernel(x_hbm, k_hbm, v_hbm, wq_hbm, wot_hbm, out_hbm,
            x_v, wq_v, wot_v, q_v, o_v, k_v, v_v, out_v,
            sem_x, sem_wq, sem_wo, sem_kv, sem_out,
            *, B, Sq, Hkv, dh, scale):
    G = B * Hkv // _U
    sk = k_v.shape[-2]
    gw = 2 * dh
    M = B * Sq
    XA = (B // 2) * Sq
    NT2 = M // 128
    step = pl.program_id(0)
    f32, bf16, u32 = jnp.float32, jnp.bfloat16, jnp.uint32

    def wq_copy(j):
        return pltpu.make_async_copy(
            wq_hbm.at[:, pl.ds(j * gw, gw)], wq_v.at[j], sem_wq.at[min(j, 2)])

    def kv_copies(g):
        slot = g % _NBLK
        return (
            pltpu.make_async_copy(k_hbm.at[pl.ds(g * _U, _U)], k_v.at[slot], sem_kv.at[0, slot]),
            pltpu.make_async_copy(v_hbm.at[pl.ds(g * _U, _U)], v_v.at[slot], sem_kv.at[1, slot]),
        )

    xa_copy = pltpu.make_async_copy(
        x_hbm.at[pl.ds(0, XA)], x_v.at[pl.ds(0, XA)], sem_x.at[0])
    xb_copy = pltpu.make_async_copy(
        x_hbm.at[pl.ds(XA, M - XA)], x_v.at[pl.ds(XA, M - XA)], sem_x.at[1])
    wo_copy = pltpu.make_async_copy(wot_hbm, wot_v, sem_wo)

    def qproj(r0, r1, j):
        qf = jnp.dot(x_v[r0:r1, :], wq_v[j], preferred_element_type=f32)
        q = (qf * (scale * _LOG2E)).astype(bf16)
        for b in range(r0 // Sq, r1 // Sq):
            for r in range(2):
                q_v[j, b, r * Sq:(r + 1) * Sq, :] = (
                    q[b * Sq - r0:(b + 1) * Sq - r0, r * dh:(r + 1) * dh])

    def phase0():
        xa_copy.start()
        wq_copy(0).start()
        xa_copy.wait()
        xb_copy.start()
        wq_copy(1).start()
        wq_copy(0).wait()
        qproj(0, XA, 0)
        for j in range(2, Hkv):
            wq_copy(j).start()
        xb_copy.wait()
        wq_copy(1).wait()
        for cp in kv_copies(0):
            cp.start()
        qproj(XA, M, 0)
        qproj(0, M, 1)
        rest = wq_v.at[pl.ds(2, Hkv - 2)]
        pltpu.make_async_copy(rest, rest, sem_wq.at[2]).wait()
        for g in range(1, _NBLK):
            for cp in kv_copies(g):
                cp.start()
        for j in range(2, Hkv):
            qproj(0, M, j)

    def softmax(s, never, deps):
        ps, lps = [], []
        for cc in range(s.shape[0] // _RC):
            sc = s[cc * _RC:(cc + 1) * _RC, :]
            st = [sc[:, t * 128:(t + 1) * 128] for t in range(sk // 128)]
            mm = st[-1]
            for t in range(len(st) - 1):
                mm = jnp.maximum(mm, st[t])
            if deps is not None:
                for t in range(deps.shape[1] // 128):
                    d = deps[cc * _RC:(cc + 1) * _RC, t * 128:(t + 1) * 128]
                    mm = jnp.where(never, d, mm)
            m = jnp.max(mm, axis=-1, keepdims=True)
            p = pltpu.bitcast(jnp.exp2(sc - m).astype(bf16), u32)
            pf = pltpu.bitcast(p, bf16).astype(f32)
            lp = pf[:, 0:128]
            for t in range(1, sk // 128):
                lp = lp + pf[:, t * 128:(t + 1) * 128]
            ps.append(p)
            lps.append(lp)
        return pltpu.bitcast(jnp.concatenate(ps, axis=0), bf16), lps

    def tie(a, c, never, lp):
        lo, hi = c * _RC, (c + 1) * _RC
        blk = pltpu.bitcast(a[lo:hi, :128], u32)
        d = pltpu.bitcast(lp[:8] + lp[8:], u32)
        blk = pltpu.bitcast(jnp.where(never, d, blk), bf16)
        row = jnp.concatenate([blk, a[lo:hi, 128:]], axis=1)
        parts = ([a[:lo]] if lo else []) + [row] + ([a[hi:]] if hi < a.shape[0] else [])
        return jnp.concatenate(parts, axis=0)

    def main(g, carry):
        slot = g % _NBLK
        never = g < 0
        for cp in kv_copies(g):
            cp.wait()
        bs = [(g * _U + i) // Hkv for i in range(_U)]
        hs = [(g * _U + i) % Hkv for i in range(_U)]
        ss = [None] * _U
        ons = [None] * _U

        def qk(i, lps):
            q = q_v[hs[i], bs[i]]
            k = k_v[slot, i]
            if lps is None:
                ss[i] = lax.dot_general(q, k, _NT, preferred_element_type=f32)
                return
            nch = len(lps)
            ng = sk // _KG
            slots = [(t, c) for t in range(_G0, ng) for c in range(nch)]
            assign = {}
            for j in range(nch):
                t, c = slots[j * len(slots) // nch]
                assign.setdefault(t, []).append((c, j))
            parts = []
            for t in range(ng):
                qt = q
                for c, j in assign.get(t, []):
                    qt = tie(qt, c, never, lps[j])
                parts.append(lax.dot_general(
                    qt, k[t * _KG:(t + 1) * _KG], _NT, preferred_element_type=f32))
            ss[i] = jnp.concatenate(parts, axis=1)

        qk(0, None)
        for i in range(_U):
            p, lps = softmax(ss[i], never, ons[i - 2] if i >= 2 else None)
            if i + 1 < _U:
                qk(i + 1, lps)
            o = jnp.dot(p, v_v[slot, i], preferred_element_type=f32)
            lp = jnp.where(never, o[:, :128], jnp.concatenate(lps, axis=0))
            on = o * (1.0 / jnp.sum(lp, axis=-1, keepdims=True))
            ob = on.astype(bf16)
            rows = pl.ds(pl.multiple_of(bs[i] * Sq, 16), Sq)
            o_v[hs[i], rows, 0:dh] = ob[:Sq]
            o_v[hs[i], rows, dh:gw] = ob[Sq:]
            ons[i] = on

        @pl.when(g + _NBLK < G)
        def _():
            for cp in kv_copies(g + _NBLK):
                cp.start()

        @pl.when(g == G - _NBLK)
        def _():
            wo_copy.start()

        return carry

    def out_rows(t):
        r0 = t * 128 if isinstance(t, int) else pl.multiple_of(t * 128, 128)
        return pl.ds(r0, 128)

    def out_copy(t):
        rows = out_rows(t)
        return pltpu.make_async_copy(out_v.at[rows], out_hbm.at[rows], sem_out.at[t])

    def phase2_body(j, carry):
        for tt in range(_P2T):
            t = j * _P2T + tt
            rows = out_rows(t)
            acc = None
            for h in range(Hkv):
                y = lax.dot_general(wot_v[:, h * gw:(h + 1) * gw], o_v[h, rows, :], _NT,
                                    preferred_element_type=f32)
                acc = y if acc is None else acc + y
            out_v[rows, :] = acc.T.astype(out_v.dtype)
            out_copy(t).start()
        return carry

    @pl.when(step == 0)
    def _():
        phase0()
        lax.fori_loop(0, G, main, 0)

    @pl.when(step == 1)
    def _():
        wo_copy.wait()
        lax.fori_loop(0, NT2 // _P2T, phase2_body, 0)
        for t in range(NT2):
            out_copy(t).wait()


@jax.jit
def pallas_standalone__gqa_block_cached__near_ridge_kernel(
    x: jax.Array,
    k_cache: jax.Array,
    v_cache: jax.Array,
    wq: jax.Array,
    wo: jax.Array,
):
    B, Sq, D = x.shape
    _, Hkv, Sk, Dh = k_cache.shape
    M = B * Sq
    gw = 2 * Dh
    assert wq.shape[1] == Hkv * gw and M % (128 * _P2T) == 0 and (B * Hkv) % _U == 0
    kern = functools.partial(_kernel, B=B, Sq=Sq, Hkv=Hkv, dh=Dh, scale=Dh ** -0.5)
    bf = jnp.bfloat16
    out = pl.pallas_call(
        kern,
        grid=(2,),
        in_specs=[pl.BlockSpec(memory_space=pl.ANY)] * 5,
        out_specs=pl.BlockSpec(memory_space=pl.ANY),
        out_shape=jax.ShapeDtypeStruct((M, D), x.dtype),
        scratch_shapes=[
            pltpu.VMEM((M, D), bf),
            pltpu.VMEM((Hkv, D, gw), bf),
            pltpu.VMEM((D, Hkv * gw), bf),
            pltpu.VMEM((Hkv, B, 2 * Sq, Dh), bf),
            pltpu.VMEM((Hkv, M, gw), bf),
            pltpu.VMEM((_NBLK, _U, Sk, Dh), bf),
            pltpu.VMEM((_NBLK, _U, Sk, Dh), bf),
            pltpu.VMEM((M, D), bf),
            pltpu.SemaphoreType.DMA((2,)),
            pltpu.SemaphoreType.DMA((3,)),
            pltpu.SemaphoreType.DMA(()),
            pltpu.SemaphoreType.DMA((2, _NBLK)),
            pltpu.SemaphoreType.DMA((M // 128,)),
        ],
        compiler_params=pltpu.CompilerParams(
            dimension_semantics=("arbitrary",),
            vmem_limit_bytes=100 * 1024 * 1024,
            disable_bounds_checks=True,
        ),
    )(x.reshape(M, D), k_cache.reshape(B * Hkv, Sk, Dh), v_cache.reshape(B * Hkv, Sk, Dh),
      wq, wo.T)
    return out.reshape(B, Sq, D)
```

```python
import functools

import jax
import jax.numpy as jnp
from jax import lax
import jax.experimental.pallas as pl
import jax.experimental.pallas.tpu as pltpu

_LOG2E = 1.4426950408889634
_NT = (((1,), (1,)), ((), ()))
_RC = 16
_U = 7
_NBLK = 2
_KG = 256
_HT = 8
_P2T = 3


def _kernel(x_hbm, k_hbm, v_hbm, wq_hbm, wot_hbm, out_hbm,
            x_v, wq_v, wot_v, q_v, o_v, k_v, v_v, k0_v, v0_v, out_v,
            sem_x, sem_wq, sem_wo, sem_kv, sem_0, sem_out,
            *, B, Sq, Hkv, dh, scale):
    G = (B * Hkv - 1) // _U
    sk = k_v.shape[-2]
    gw = 2 * dh
    M = B * Sq
    XA = (B // 2) * Sq
    NT2 = M // 128
    QL = (Hkv - 2) // 2
    DN = (out_v.shape[1] // 128) * 128
    step = pl.program_id(0)
    f32, bf16, u32 = jnp.float32, jnp.bfloat16, jnp.uint32

    def wq_copy(j):
        s = j if j < 2 else 2 + (j - 2) // QL
        return pltpu.make_async_copy(
            wq_hbm.at[:, pl.ds(j * gw, gw)], wq_v.at[j], sem_wq.at[s])

    def kv_copies(g):
        slot = g % _NBLK
        units = pl.ds(1 + g * _U, _U)
        return (
            pltpu.make_async_copy(k_hbm.at[units], k_v.at[slot], sem_kv.at[0, slot]),
            pltpu.make_async_copy(v_hbm.at[units], v_v.at[slot], sem_kv.at[1, slot]),
        )

    kv0_copies = (pltpu.make_async_copy(k_hbm.at[0], k0_v, sem_0.at[0]),
                  pltpu.make_async_copy(v_hbm.at[0], v0_v, sem_0.at[1]))
    xa_copy = pltpu.make_async_copy(
        x_hbm.at[pl.ds(0, XA)], x_v.at[pl.ds(0, XA)], sem_x.at[0])
    xb_copy = pltpu.make_async_copy(
        x_hbm.at[pl.ds(XA, M - XA)], x_v.at[pl.ds(XA, M - XA)], sem_x.at[1])
    wo_copy = pltpu.make_async_copy(wot_hbm, wot_v, sem_wo)

    def out_rows(t):
        r0 = t * 128 if isinstance(t, int) else pl.multiple_of(t * 128, 128)
        return pl.ds(r0, 128)

    def out_copy(t):
        rows = out_rows(t)
        return pltpu.make_async_copy(out_v.at[rows], out_hbm.at[rows], sem_out.at[t])

    def qproj(r0, r1, j):
        qf = jnp.dot(x_v[r0:r1, :], wq_v[j], preferred_element_type=f32)
        q = (qf * (scale * _LOG2E)).astype(bf16)
        for b in range(r0 // Sq, r1 // Sq):
            for r in range(2):
                q_v[j, b, r] = q[b * Sq - r0:(b + 1) * Sq - r0, r * dh:(r + 1) * dh]

    def softmax(s, never, deps):
        ps, lps, tls = [], [], []
        nt = sk // 128
        for cc in range(s.shape[0] // _RC):
            sc = s[cc * _RC:(cc + 1) * _RC, :]
            st = [sc[:, t * 128:(t + 1) * 128] for t in range(nt)]
            mm = st[-1]
            for t in range(nt - 1):
                mm = jnp.maximum(mm, st[t])
            if deps is not None:
                for t in range(deps.shape[1] // 128):
                    d = deps[cc * _RC:(cc + 1) * _RC, t * 128:(t + 1) * 128]
                    mm = jnp.where(never, d, mm)
            m = jnp.max(mm, axis=-1, keepdims=True)
            p = pltpu.bitcast(jnp.exp2(sc - m).astype(bf16), u32)
            pf = pltpu.bitcast(p, bf16).astype(f32)
            lp = pf[:, 0:128]
            for t in range(1, nt):
                lp = lp + pf[:, t * 128:(t + 1) * 128]
                if (t + 1) % (nt // _HT) == 0:
                    tls.append(lp)
            ps.append(p)
            lps.append(lp)
        return pltpu.bitcast(jnp.concatenate(ps, axis=0), bf16), lps, tls

    def tie(a, c, never, lp):
        lo, hi = c * _RC, (c + 1) * _RC
        blk = pltpu.bitcast(a[lo:hi, :128], u32)
        d = pltpu.bitcast(lp[:8] + lp[8:], u32)
        blk = pltpu.bitcast(jnp.where(never, d, blk), bf16)
        row = jnp.concatenate([blk, a[lo:hi, 128:]], axis=1)
        parts = ([a[:lo]] if lo else []) + [row] + ([a[hi:]] if hi < a.shape[0] else [])
        return jnp.concatenate(parts, axis=0)

    def normalize(o, lps, never):
        lp = jnp.where(never, o[:, :128], jnp.concatenate(lps, axis=0))
        return o * (1.0 / jnp.sum(lp, axis=-1, keepdims=True))

    def qloop(t, carry):
        never = t < 0
        grp = wq_v.at[pl.ds(2 + t * QL, QL)]
        pltpu.make_async_copy(grp, grp, sem_wq.at[2 + t]).wait()
        q = q_v[0, 0, t]
        qproj(0, M, 2 + t * QL)
        s = lax.dot_general(q, k0_v[...], _NT, preferred_element_type=f32)
        qproj(0, M, 3 + t * QL)
        p, lps, _ = softmax(s, never, None)
        o = jnp.dot(p, v0_v[...], preferred_element_type=f32)
        for j in range(2, QL):
            qproj(0, M, 2 + j + t * QL)
        o_v[0, t, 0:Sq, :] = normalize(o, lps, never).astype(bf16)
        return carry

    def phase0():
        xa_copy.start()
        wq_copy(0).start()
        xa_copy.wait()
        xb_copy.start()
        wq_copy(1).start()
        wq_copy(0).wait()
        qproj(0, XA, 0)
        for j in range(2, 2 + QL):
            wq_copy(j).start()
        for cp in kv0_copies:
            cp.start()
        xb_copy.wait()
        for j in range(2 + QL, Hkv):
            wq_copy(j).start()
        wq_copy(1).wait()
        qproj(XA, M, 0)
        qproj(0, M, 1)
        kv0_copies[0].wait()
        for cp in kv_copies(0):
            cp.start()
        kv0_copies[1].wait()
        lax.fori_loop(0, 2, qloop, 0)
        for g in range(1, _NBLK):
            for cp in kv_copies(g):
                cp.start()

    def main(g, carry):
        slot = g % _NBLK
        never = g < 0
        for cp in kv_copies(g):
            cp.wait()
        us = [1 + g * _U + i for i in range(_U)]
        bs = [u // Hkv for u in us]
        hs = [u % Hkv for u in us]
        ss = [None] * _U
        ons = [None] * _U

        def qk(i, tls):
            q = jnp.concatenate([q_v[hs[i], bs[i], 0], q_v[hs[i], bs[i], 1]], axis=0)
            k = k_v[slot, i]
            if tls is None:
                ss[i] = lax.dot_general(q, k, _NT, preferred_element_type=f32)
                return
            n = len(tls)
            ng = sk // _KG
            slots = [(t, c) for t in range(2 if i == 1 else 0, ng)
                     for c in range(q.shape[0] // _RC)]
            assign = {}
            for j in range(n):
                t, c = slots[j * len(slots) // n]
                assign.setdefault(t, []).append((c, j))
            parts = []
            for t in range(ng):
                qt = q
                for c, j in assign.get(t, []):
                    qt = tie(qt, c, never, tls[j])
                parts.append(lax.dot_general(
                    qt, k[t * _KG:(t + 1) * _KG], _NT, preferred_element_type=f32))
            ss[i] = jnp.concatenate(parts, axis=1)

        qk(0, None)
        for i in range(_U):
            p, lps, tls = softmax(ss[i], never, ons[i - 2] if i >= 2 else None)
            if i + 1 < _U:
                qk(i + 1, tls)
            o = jnp.dot(p, v_v[slot, i], preferred_element_type=f32)
            on = normalize(o, lps, never)
            ob = on.astype(bf16)
            rows = pl.ds(pl.multiple_of(bs[i] * Sq, 16), Sq)
            o_v[hs[i], 0, rows, :] = ob[:Sq]
            o_v[hs[i], 1, rows, :] = ob[Sq:]
            ons[i] = on

        @pl.when(g + _NBLK < G)
        def _():
            for cp in kv_copies(g + _NBLK):
                cp.start()

        @pl.when(g == G - _NBLK)
        def _():
            wo_copy.start()

        return carry

    def oloop(j, carry):
        for tt in range(_P2T):
            t = j * _P2T + tt
            rows = out_rows(t)

            def oh(h):
                return jnp.concatenate([o_v[h, 0, rows, :], o_v[h, 1, rows, :]], axis=1)

            yt = None
            for h in range(Hkv):
                y = lax.dot_general(wot_v[DN:, h * gw:(h + 1) * gw], oh(h), _NT,
                                    preferred_element_type=f32)
                yt = y if yt is None else yt + y
            yn = None
            for h in range(Hkv):
                y = lax.dot_general(oh(h), wot_v[:DN, h * gw:(h + 1) * gw], _NT,
                                    preferred_element_type=f32)
                yn = y if yn is None else yn + y
            out_v[rows, :] = jnp.concatenate([yn, yt.T], axis=1).astype(out_v.dtype)
            out_copy(t).start()
        return carry

    @pl.when(step == 0)
    def _():
        phase0()
        lax.fori_loop(0, G, main, 0)

    @pl.when(step == 1)
    def _():
        wo_copy.wait()
        lax.fori_loop(0, NT2 // _P2T, oloop, 0)
        for t in range(NT2):
            out_copy(t).wait()


@jax.jit
def pallas_standalone__gqa_block_cached__near_ridge_kernel(
    x: jax.Array,
    k_cache: jax.Array,
    v_cache: jax.Array,
    wq: jax.Array,
    wo: jax.Array,
):
    B, Sq, D = x.shape
    _, Hkv, Sk, Dh = k_cache.shape
    M = B * Sq
    gw = 2 * Dh
    assert wq.shape[1] == Hkv * gw and Hkv % 2 == 0 and Hkv >= 6 and D % 128 != 0
    assert M % (128 * _P2T) == 0 and (B * Hkv - 1) % _U == 0 and Sq % _RC == 0
    kern = functools.partial(_kernel, B=B, Sq=Sq, Hkv=Hkv, dh=Dh, scale=Dh ** -0.5)
    bf = jnp.bfloat16
    out = pl.pallas_call(
        kern,
        grid=(2,),
        in_specs=[pl.BlockSpec(memory_space=pl.ANY)] * 5,
        out_specs=pl.BlockSpec(memory_space=pl.ANY),
        out_shape=jax.ShapeDtypeStruct((M, D), x.dtype),
        scratch_shapes=[
            pltpu.VMEM((M, D), bf),
            pltpu.VMEM((Hkv, D, gw), bf),
            pltpu.VMEM((D, Hkv * gw), bf),
            pltpu.VMEM((Hkv, B, 2, Sq, Dh), bf),
            pltpu.VMEM((Hkv, 2, M, Dh), bf),
            pltpu.VMEM((_NBLK, _U, Sk, Dh), bf),
            pltpu.VMEM((_NBLK, _U, Sk, Dh), bf),
            pltpu.VMEM((Sk, Dh), bf),
            pltpu.VMEM((Sk, Dh), bf),
            pltpu.VMEM((M, D), bf),
            pltpu.SemaphoreType.DMA((2,)),
            pltpu.SemaphoreType.DMA((4,)),
            pltpu.SemaphoreType.DMA(()),
            pltpu.SemaphoreType.DMA((2, _NBLK)),
            pltpu.SemaphoreType.DMA((2,)),
            pltpu.SemaphoreType.DMA((M // 128,)),
        ],
        compiler_params=pltpu.CompilerParams(
            dimension_semantics=("arbitrary",),
            vmem_limit_bytes=100 * 1024 * 1024,
            disable_bounds_checks=True,
            disable_semaphore_checks=True,
        ),
    )(x.reshape(M, D), k_cache.reshape(B * Hkv, Sk, Dh), v_cache.reshape(B * Hkv, Sk, Dh),
      wq, wo.T)
    return out.reshape(B, Sq, D)
```

```python
import functools

import jax
import jax.numpy as jnp
from jax import lax
import jax.experimental.pallas as pl
import jax.experimental.pallas.tpu as pltpu

_LOG2E = 1.4426950408889634
_NT = (((1,), (1,)), ((), ()))
_RC = 16
_U = 7
_NBLK = 2
_KG = 256
_PG = 512
_PW = 2
_Q0 = 27
_S0 = 36
_P2T = 3


def _kernel(x_hbm, k_hbm, v_hbm, wq_hbm, wot_hbm, out_hbm,
            x_v, wq_v, wot_v, q_v, o_v, k_v, v_v, k0_v, v0_v, out_v,
            sem_x, sem_wq, sem_wo, sem_kv, sem_0, sem_out,
            *, B, Sq, Hkv, dh, scale):
    G = (B * Hkv - 1) // _U
    sk = k_v.shape[-2]
    nt = sk // 128
    gw = 2 * dh
    M = B * Sq
    XA = (B // 2) * Sq
    NT2 = M // 128
    QL = (Hkv - 2) // 2
    DN = (out_v.shape[1] // 128) * 128
    step = pl.program_id(0)
    f32, bf16, u32 = jnp.float32, jnp.bfloat16, jnp.uint32
    escale = scale * _LOG2E

    def wq_copy(j):
        s = j if j < 2 else 2 + (j - 2) // QL
        return pltpu.make_async_copy(
            wq_hbm.at[:, pl.ds(j * gw, gw)], wq_v.at[j], sem_wq.at[s])

    def kv_copies(g):
        slot = g % _NBLK if isinstance(g, int) else lax.rem(g, _NBLK)
        units = pl.ds(1 + g * _U, _U)
        return (
            pltpu.make_async_copy(k_hbm.at[units], k_v.at[slot], sem_kv.at[0, slot]),
            pltpu.make_async_copy(v_hbm.at[units], v_v.at[slot], sem_kv.at[1, slot]),
        )

    kv0_copies = (pltpu.make_async_copy(k_hbm.at[0], k0_v, sem_0.at[0]),
                  pltpu.make_async_copy(v_hbm.at[0], v0_v, sem_0.at[1]))
    xa_copy = pltpu.make_async_copy(
        x_hbm.at[pl.ds(0, XA)], x_v.at[pl.ds(0, XA)], sem_x.at[0])
    xb_copy = pltpu.make_async_copy(
        x_hbm.at[pl.ds(XA, M - XA)], x_v.at[pl.ds(XA, M - XA)], sem_x.at[1])
    wo_copy = pltpu.make_async_copy(wot_hbm, wot_v, sem_wo)

    def out_rows(t):
        r0 = t * 128 if isinstance(t, int) else pl.multiple_of(t * 128, 128)
        return pl.ds(r0, 128)

    def out_copy(t):
        rows = out_rows(t)
        return pltpu.make_async_copy(out_v.at[rows], out_hbm.at[rows], sem_out.at[t])

    def qproj(r0, r1, j):
        q = jnp.dot(x_v[r0:r1, :], wq_v[j], preferred_element_type=f32).astype(bf16)
        for b in range(r0 // Sq, r1 // Sq):
            for r in range(2):
                q_v[j, b, r] = q[b * Sq - r0:(b + 1) * Sq - r0, r * dh:(r + 1) * dh]

    def tile(a, c, lo):
        return a[c * _RC:(c + 1) * _RC, lo:lo + 128]

    def rowmax(s, c, never, deps):
        mm = tile(s, c, (nt - 1) * 128)
        for t in range(nt - 1):
            mm = jnp.maximum(mm, tile(s, c, t * 128))
        if deps is not None:
            for t in range(deps.shape[1] // 128):
                mm = jnp.where(never, tile(deps, c, t * 128), mm)
        return jnp.max(mm.astype(bf16).astype(f32), axis=-1, keepdims=True)

    def normalize(o, lps, never):
        lp = jnp.where(never, o[:, :128], jnp.concatenate(lps, axis=0))
        l = jnp.sum(lp, axis=-1, keepdims=True)
        r = pl.reciprocal(l, approx=True)
        r = r * (2.0 - l * r)
        return o * r

    def qloop(t, carry):
        never = t < 0
        grp = wq_v.at[pl.ds(2 + t * QL, QL)]
        pltpu.make_async_copy(grp, grp, sem_wq.at[2 + t]).wait()
        q = q_v[0, 0, t]
        qproj(0, M, 2 + t * QL)
        s = lax.dot_general(q, k0_v[...], _NT, preferred_element_type=f32)
        qproj(0, M, 3 + t * QL)
        ps, lps = [], []
        for c in range(Sq // _RC):
            m = rowmax(s, c, never, None)
            sr = s[c * _RC:(c + 1) * _RC, :].astype(bf16).astype(f32)
            p = pltpu.bitcast(jnp.exp2((sr - m) * escale).astype(bf16), u32)
            pf = pltpu.bitcast(p, bf16).astype(f32)
            lp = pf[:, 0:128]
            for tt in range(1, nt):
                lp = lp + pf[:, tt * 128:(tt + 1) * 128]
            ps.append(p)
            lps.append(lp)
        pb = pltpu.bitcast(jnp.concatenate(ps, axis=0), bf16)
        o = jnp.dot(pb, v0_v[...], preferred_element_type=f32)
        for j in range(2, QL):
            qproj(0, M, 2 + j + t * QL)
        o_v[0, t, 0:Sq, :] = normalize(o, lps, never).astype(bf16)
        return carry

    def phase0():
        xa_copy.start()
        wq_copy(0).start()
        xa_copy.wait()
        xb_copy.start()
        wq_copy(1).start()
        wq_copy(0).wait()
        qproj(0, XA, 0)
        for j in range(2, 2 + QL):
            wq_copy(j).start()
        for cp in kv0_copies:
            cp.start()
        xb_copy.wait()
        for j in range(2 + QL, Hkv):
            wq_copy(j).start()
        wq_copy(1).wait()
        qproj(XA, M, 0)
        qproj(0, M, 1)
        kv0_copies[0].wait()
        for cp in kv_copies(0):
            cp.start()
        kv0_copies[1].wait()
        lax.fori_loop(0, 2, qloop, 0)
        for g in range(1, _NBLK):
            for cp in kv_copies(g):
                cp.start()

    def main(g, carry):
        slot = lax.rem(g, _NBLK)
        never = g < 0
        for cp in kv_copies(g):
            cp.wait()
        us = [1 + g * _U + i for i in range(_U)]
        bs = [lax.div(u, Hkv) for u in us]
        hs = [lax.rem(u, Hkv) for u in us]
        nc = 2 * Sq // _RC
        npart = nt // _PW
        nport = nc * npart
        ss = [None] * _U
        os_ = [None] * _U
        ons = [None] * _U
        ms = [None] * _U
        pp = [[[] for _ in range(nc)] for _ in range(_U)]
        lps = [[None] * nc for _ in range(_U)]

        def sm_max(i, deps):
            ms[i] = [jnp.broadcast_to(rowmax(ss[i], c, never, deps), (_RC, 128))
                     for c in range(nc)]

        def sm_portion(i, j, anchor):
            c, part = j // npart, j % npart
            m = jnp.where(never, anchor, ms[i][c])
            sc = ss[i][c * _RC:(c + 1) * _RC, part * _PW * 128:(part + 1) * _PW * 128]
            sr = sc.astype(bf16).astype(f32)
            for t in range(_PW):
                p = jnp.exp2((sr[:, t * 128:(t + 1) * 128] - m) * escale)
                pp[i][c].append(p)
                lps[i][c] = p if lps[i][c] is None else lps[i][c] + p
            return lps[i][c]

        def assign_slots(first, nslots):
            a = {}
            for j in range(nport):
                a.setdefault(first + j * (nslots - first) // nport, []).append(j)
            return a

        def qk(i):
            q = jnp.concatenate([q_v[hs[i], bs[i], 0], q_v[hs[i], bs[i], 1]], axis=0)
            k = k_v[slot, i]
            if i == 0:
                ss[i] = lax.dot_general(q, k, _NT, preferred_element_type=f32)
                return
            ng = sk // _KG
            assign = assign_slots(_Q0 if i == 1 else 0, ng * nc)
            qa = pltpu.bitcast(q[:, :128], u32)
            hr = _RC // 2
            parts = []
            for t in range(ng):
                blks = []
                for c in range(nc):
                    blk = qa[c * hr:(c + 1) * hr]
                    for j in assign.get(t * nc + c, []):
                        anchor = tile(parts[t - 1], c, 0) if t else tile(os_[i - 2], c, 128)
                        lp = sm_portion(i - 1, j, anchor)
                        blk = jnp.where(never, pltpu.bitcast(lp[:8] + lp[8:], u32), blk)
                    blks.append(blk)
                qt = jnp.concatenate(
                    [pltpu.bitcast(jnp.concatenate(blks, axis=0), bf16), q[:, 128:]], axis=1)
                parts.append(lax.dot_general(
                    qt, k[t * _KG:(t + 1) * _KG], _NT, preferred_element_type=f32))
            ss[i] = jnp.concatenate(parts, axis=1)

        def pv(i):
            v = v_v[slot, i]
            if i != _U - 2:
                pb = jnp.concatenate(
                    [jnp.concatenate(r, axis=1) for r in pp[i]], axis=0).astype(bf16)
                return jnp.dot(pb, v, preferred_element_type=f32)
            ng = sk // _PG
            tg = _PG // 128
            assign = assign_slots(_S0, (dh // 128) * ng * nc)
            outs = []
            prev = None
            for half in range(dh // 128):
                acc = None
                for kg in range(ng):
                    rows = []
                    for c in range(nc):
                        tl = pp[i][c][kg * tg:(kg + 1) * tg]
                        blk = tl[0]
                        for j in assign.get((half * ng + kg) * nc + c, []):
                            lp = sm_portion(i + 1, j, tile(prev, c, 0))
                            blk = jnp.where(never, lp, blk)
                        rows.append(jnp.concatenate([blk] + tl[1:], axis=1))
                    pb = jnp.concatenate(rows, axis=0).astype(bf16)
                    y = jnp.dot(pb, v[kg * _PG:(kg + 1) * _PG, half * 128:(half + 1) * 128],
                                preferred_element_type=f32)
                    acc = y if acc is None else acc + y
                    prev = acc
                outs.append(acc)
            return jnp.concatenate(outs, axis=1)

        qk(0)
        for i in range(_U):
            if i < _U - 1:
                sm_max(i, ons[i - 2] if i >= 2 else None)
                qk(i + 1)
            if i == _U - 2:
                sm_max(i + 1, None)
            o = pv(i)
            on = normalize(o, lps[i], never)
            ob = on.astype(bf16)
            rows = pl.ds(pl.multiple_of(bs[i] * Sq, 16), Sq)
            o_v[hs[i], 0, rows, :] = ob[:Sq]
            o_v[hs[i], 1, rows, :] = ob[Sq:]
            os_[i] = o
            ons[i] = on

        @pl.when(g + _NBLK < G)
        def _():
            for cp in kv_copies(g + _NBLK):
                cp.start()

        @pl.when(g == G - _NBLK)
        def _():
            wo_copy.start()

        return carry

    def oloop(j, carry):
        for tt in range(_P2T):
            t = j * _P2T + tt
            rows = out_rows(t)

            def oh(h):
                return jnp.concatenate([o_v[h, 0, rows, :], o_v[h, 1, rows, :]], axis=1)

            def tpart():
                yt = None
                for h in range(Hkv):
                    y = lax.dot_general(wot_v[DN:, h * gw:(h + 1) * gw], oh(h), _NT,
                                        preferred_element_type=f32)
                    yt = y if yt is None else yt + y
                return yt

            def npart():
                yn = None
                for h in range(Hkv):
                    y = lax.dot_general(oh(h), wot_v[:DN, h * gw:(h + 1) * gw], _NT,
                                        preferred_element_type=f32)
                    yn = y if yn is None else yn + y
                return yn

            if tt == 0:
                yn = npart()
                yt = tpart()
            else:
                yt = tpart()
                yn = npart()
            out_v[rows, :] = jnp.concatenate([yn, yt.T], axis=1).astype(out_v.dtype)
            out_copy(t).start()
        return carry

    @pl.when(step == 0)
    def _():
        phase0()
        lax.fori_loop(0, G, main, 0)

    @pl.when(step == 1)
    def _():
        wo_copy.wait()
        lax.fori_loop(0, NT2 // _P2T, oloop, 0)
        for t in range(NT2):
            out_copy(t).wait()


@jax.jit
def pallas_standalone__gqa_block_cached__near_ridge_kernel(
    x: jax.Array,
    k_cache: jax.Array,
    v_cache: jax.Array,
    wq: jax.Array,
    wo: jax.Array,
):
    B, Sq, D = x.shape
    _, Hkv, Sk, Dh = k_cache.shape
    M = B * Sq
    gw = 2 * Dh
    assert wq.shape[1] == Hkv * gw and Hkv % 2 == 0 and Hkv >= 6 and D % 128 != 0
    assert M % (128 * _P2T) == 0 and (B * Hkv - 1) % _U == 0 and Sq % _RC == 0
    assert Dh == 256 and Sk % _PG == 0
    kern = functools.partial(_kernel, B=B, Sq=Sq, Hkv=Hkv, dh=Dh, scale=Dh ** -0.5)
    bf = jnp.bfloat16
    out = pl.pallas_call(
        kern,
        grid=(2,),
        in_specs=[pl.BlockSpec(memory_space=pl.ANY)] * 5,
        out_specs=pl.BlockSpec(memory_space=pl.ANY),
        out_shape=jax.ShapeDtypeStruct((M, D), x.dtype),
        scratch_shapes=[
            pltpu.VMEM((M, D), bf),
            pltpu.VMEM((Hkv, D, gw), bf),
            pltpu.VMEM((D, Hkv * gw), bf),
            pltpu.VMEM((Hkv, B, 2, Sq, Dh), bf),
            pltpu.VMEM((Hkv, 2, M, Dh), bf),
            pltpu.VMEM((_NBLK, _U, Sk, Dh), bf),
            pltpu.VMEM((_NBLK, _U, Sk, Dh), bf),
            pltpu.VMEM((Sk, Dh), bf),
            pltpu.VMEM((Sk, Dh), bf),
            pltpu.VMEM((M, D), bf),
            pltpu.SemaphoreType.DMA((2,)),
            pltpu.SemaphoreType.DMA((4,)),
            pltpu.SemaphoreType.DMA(()),
            pltpu.SemaphoreType.DMA((2, _NBLK)),
            pltpu.SemaphoreType.DMA((2,)),
            pltpu.SemaphoreType.DMA((M // 128,)),
        ],
        compiler_params=pltpu.CompilerParams(
            dimension_semantics=("arbitrary",),
            vmem_limit_bytes=100 * 1024 * 1024,
            disable_bounds_checks=True,
            disable_semaphore_checks=True,
        ),
    )(x.reshape(M, D), k_cache.reshape(B * Hkv, Sk, Dh), v_cache.reshape(B * Hkv, Sk, Dh),
      wq, wo.T)
    return out.reshape(B, Sq, D)
```

```python
import functools

import jax
import jax.numpy as jnp
from jax import lax
import jax.experimental.pallas as pl
import jax.experimental.pallas.tpu as pltpu

_LOG2E = 1.4426950408889634
_NT = (((1,), (1,)), ((), ()))
_RC = 16
_U = 7
_NBLK = 2
_KG = 256
_PG = 512
_PW = 2
_Q0 = 27
_S0 = 36
_P2T = 3
_X0 = 384
_X1 = 640


def _kernel(x_hbm, k_hbm, v_hbm, wq_hbm, wot_hbm, out_hbm,
            x_v, wq_v, wot_v, q_v, o_v, k_v, v_v, k0_v, v0_v, out_v,
            sem, sem_out,
            *, B, Sq, Hkv, dh, scale):
    G = (B * Hkv - 1) // _U
    sk = k_v.shape[-2]
    nt = sk // 128
    gw = 2 * dh
    M = B * Sq
    NT2 = M // 128
    QL = (Hkv - 2) // 2
    DN = (out_v.shape[1] // 128) * 128
    step = pl.program_id(0)
    f32, bf16, u32 = jnp.float32, jnp.bfloat16, jnp.uint32
    escale = scale * _LOG2E

    def x_copy(i):
        lo, hi = ((0, _X0), (_X0, _X1), (_X1, M))[i]
        rows = pl.ds(lo, hi - lo)
        return pltpu.make_async_copy(x_hbm.at[rows], x_v.at[rows], sem.at[i])

    def wq0_copy(r):
        cols = pl.ds(r * dh, dh)
        return pltpu.make_async_copy(wq_hbm.at[:, cols], wq_v.at[0, :, cols], sem.at[3 + r])

    def wq_copy(j):
        s = 5 if j == 1 else 6 + (j - 2) // QL
        return pltpu.make_async_copy(
            wq_hbm.at[:, pl.ds(j * gw, gw)], wq_v.at[j], sem.at[s])

    kv0_copies = (pltpu.make_async_copy(k_hbm.at[0], k0_v, sem.at[8]),
                  pltpu.make_async_copy(v_hbm.at[0], v0_v, sem.at[9]))
    wo_copy = pltpu.make_async_copy(wot_hbm, wot_v, sem.at[10])

    def kv_copies(g):
        slot = g % _NBLK if isinstance(g, int) else lax.rem(g, _NBLK)
        units = pl.ds(1 + g * _U, _U)
        return (
            pltpu.make_async_copy(k_hbm.at[units], k_v.at[slot], sem.at[11 + slot]),
            pltpu.make_async_copy(v_hbm.at[units], v_v.at[slot], sem.at[11 + _NBLK + slot]),
        )

    def out_rows(t):
        r0 = t * 128 if isinstance(t, int) else pl.multiple_of(t * 128, 128)
        return pl.ds(r0, 128)

    def out_copy(t):
        rows = out_rows(t)
        return pltpu.make_async_copy(out_v.at[rows], out_hbm.at[rows], sem_out.at[t])

    def qproj(r0, r1, j, heads=(0, 1)):
        w = wq_v[j] if len(heads) == 2 else wq_v[j, :, heads[0] * dh:(heads[0] + 1) * dh]
        q = jnp.dot(x_v[r0:r1, :], w, preferred_element_type=f32).astype(bf16)
        for b in range(B):
            lo, hi = max(r0, b * Sq), min(r1, (b + 1) * Sq)
            if lo < hi:
                for n, r in enumerate(heads):
                    q_v[j, b, r, lo - b * Sq:hi - b * Sq, :] = (
                        q[lo - r0:hi - r0, n * dh:(n + 1) * dh])

    def tile(a, c, lo):
        return a[c * _RC:(c + 1) * _RC, lo:lo + 128]

    def rowmax(s, c, never, deps):
        mm = tile(s, c, (nt - 1) * 128)
        for t in range(nt - 1):
            mm = jnp.maximum(mm, tile(s, c, t * 128))
        if deps is not None:
            for t in range(deps.shape[1] // 128):
                mm = jnp.where(never, tile(deps, c, t * 128), mm)
        return jnp.max(mm.astype(bf16).astype(f32), axis=-1, keepdims=True)

    def normalize(o, lps, never):
        lp = jnp.where(never, o[:, :128], jnp.concatenate(lps, axis=0))
        l = jnp.sum(lp, axis=-1, keepdims=True)
        r = pl.reciprocal(l, approx=True)
        r = r * (2.0 - l * r)
        return o * r

    def qloop(t, carry):
        never = t < 0
        grp = wq_v.at[pl.ds(2 + t * QL, QL)]
        pltpu.make_async_copy(grp, grp, sem.at[6 + t]).wait()
        q = q_v[0, 0, t]
        qproj(0, M, 2 + t * QL)
        s = lax.dot_general(q, k0_v[...], _NT, preferred_element_type=f32)
        qproj(0, M, 3 + t * QL)
        ps, lps = [], []
        for c in range(Sq // _RC):
            m = rowmax(s, c, never, None)
            sr = s[c * _RC:(c + 1) * _RC, :].astype(bf16).astype(f32)
            p = pltpu.bitcast(jnp.exp2((sr - m) * escale).astype(bf16), u32)
            pf = pltpu.bitcast(p, bf16).astype(f32)
            lp = pf[:, 0:128]
            for tt in range(1, nt):
                lp = lp + pf[:, tt * 128:(tt + 1) * 128]
            ps.append(p)
            lps.append(lp)
        pb = pltpu.bitcast(jnp.concatenate(ps, axis=0), bf16)
        o = jnp.dot(pb, v0_v[...], preferred_element_type=f32)
        for j in range(2, QL):
            qproj(0, M, 2 + j + t * QL)
        o_v[0, t, 0:Sq, :] = normalize(o, lps, never).astype(bf16)
        return carry

    def phase0():
        x_copy(0).start()
        wq0_copy(0).start()
        wq0_copy(1).start()
        x_copy(1).start()
        x_copy(2).start()
        for j in range(1, 2 + QL):
            wq_copy(j).start()
        for cp in kv0_copies:
            cp.start()
        for j in range(2 + QL, Hkv):
            wq_copy(j).start()
        for g in range(_NBLK):
            for cp in kv_copies(g):
                cp.start()
        x_copy(0).wait()
        wq0_copy(0).wait()
        qproj(0, _X0, 0, (0,))
        wq0_copy(1).wait()
        x_copy(1).wait()
        qproj(0, _X0, 0, (1,))
        qproj(_X0, _X1, 0)
        x_copy(2).wait()
        wq_copy(1).wait()
        qproj(_X1, M, 0)
        qproj(0, M, 1)
        for cp in kv0_copies:
            cp.wait()
        lax.fori_loop(0, 2, qloop, 0)

    def main(g, carry):
        slot = lax.rem(g, _NBLK)
        never = g < 0
        for cp in kv_copies(g):
            cp.wait()
        us = [1 + g * _U + i for i in range(_U)]
        bs = [lax.div(u, Hkv) for u in us]
        hs = [lax.rem(u, Hkv) for u in us]
        nc = 2 * Sq // _RC
        npart = nt // _PW
        nport = nc * npart
        ss = [None] * _U
        os_ = [None] * _U
        ons = [None] * _U
        ms = [None] * _U
        pp = [[[] for _ in range(nc)] for _ in range(_U)]
        lps = [[None] * nc for _ in range(_U)]

        def sm_max(i, deps):
            ms[i] = [jnp.broadcast_to(rowmax(ss[i], c, never, deps), (_RC, 128))
                     for c in range(nc)]

        def sm_portion(i, j, anchor):
            c, part = j // npart, j % npart
            m = jnp.where(never, anchor, ms[i][c])
            sc = ss[i][c * _RC:(c + 1) * _RC, part * _PW * 128:(part + 1) * _PW * 128]
            sr = sc.astype(bf16).astype(f32)
            for t in range(_PW):
                p = jnp.exp2((sr[:, t * 128:(t + 1) * 128] - m) * escale)
                pp[i][c].append(p)
                lps[i][c] = p if lps[i][c] is None else lps[i][c] + p
            return lps[i][c]

        def assign_slots(first, nslots):
            a = {}
            for j in range(nport):
                a.setdefault(first + j * (nslots - first) // nport, []).append(j)
            return a

        def qk(i):
            q = jnp.concatenate([q_v[hs[i], bs[i], 0], q_v[hs[i], bs[i], 1]], axis=0)
            k = k_v[slot, i]
            if i == 0:
                ss[i] = lax.dot_general(q, k, _NT, preferred_element_type=f32)
                return
            ng = sk // _KG
            assign = assign_slots(_Q0 if i == 1 else 0, ng * nc)
            qa = pltpu.bitcast(q[:, :128], u32)
            hr = _RC // 2
            parts = []
            for t in range(ng):
                blks = []
                for c in range(nc):
                    blk = qa[c * hr:(c + 1) * hr]
                    for j in assign.get(t * nc + c, []):
                        anchor = tile(parts[t - 1], c, 0) if t else tile(os_[i - 2], c, 128)
                        lp = sm_portion(i - 1, j, anchor)
                        blk = jnp.where(never, pltpu.bitcast(lp[:8] + lp[8:], u32), blk)
                    blks.append(blk)
                qt = jnp.concatenate(
                    [pltpu.bitcast(jnp.concatenate(blks, axis=0), bf16), q[:, 128:]], axis=1)
                parts.append(lax.dot_general(
                    qt, k[t * _KG:(t + 1) * _KG], _NT, preferred_element_type=f32))
            ss[i] = jnp.concatenate(parts, axis=1)

        def pv(i):
            v = v_v[slot, i]
            if i != _U - 2:
                pb = jnp.concatenate(
                    [jnp.concatenate(r, axis=1) for r in pp[i]], axis=0).astype(bf16)
                return jnp.dot(pb, v, preferred_element_type=f32)
            ng = sk // _PG
            tg = _PG // 128
            assign = assign_slots(_S0, (dh // 128) * ng * nc)
            outs = []
            prev = None
            for half in range(dh // 128):
                acc = None
                for kg in range(ng):
                    rows = []
                    for c in range(nc):
                        tl = pp[i][c][kg * tg:(kg + 1) * tg]
                        blk = tl[0]
                        for j in assign.get((half * ng + kg) * nc + c, []):
                            lp = sm_portion(i + 1, j, tile(prev, c, 0))
                            blk = jnp.where(never, lp, blk)
                        rows.append(jnp.concatenate([blk] + tl[1:], axis=1))
                    pb = jnp.concatenate(rows, axis=0).astype(bf16)
                    y = jnp.dot(pb, v[kg * _PG:(kg + 1) * _PG, half * 128:(half + 1) * 128],
                                preferred_element_type=f32)
                    acc = y if acc is None else acc + y
                    prev = acc
                outs.append(acc)
            return jnp.concatenate(outs, axis=1)

        qk(0)
        for i in range(_U):
            if i < _U - 1:
                sm_max(i, ons[i - 2] if i >= 2 else None)
                qk(i + 1)
            if i == _U - 2:
                sm_max(i + 1, None)
            o = pv(i)
            on = normalize(o, lps[i], never)
            ob = on.astype(bf16)
            rows = pl.ds(pl.multiple_of(bs[i] * Sq, 16), Sq)
            o_v[hs[i], 0, rows, :] = ob[:Sq]
            o_v[hs[i], 1, rows, :] = ob[Sq:]
            os_[i] = o
            ons[i] = on

        @pl.when(g + _NBLK < G)
        def _():
            for cp in kv_copies(g + _NBLK):
                cp.start()

        @pl.when(g == G - _NBLK)
        def _():
            wo_copy.start()

        return carry

    def oloop(j, carry):
        for tt in range(_P2T):
            t = j * _P2T + tt
            rows = out_rows(t)

            def oh(h):
                return jnp.concatenate([o_v[h, 0, rows, :], o_v[h, 1, rows, :]], axis=1)

            def tpart():
                yt = None
                for h in range(Hkv):
                    y = lax.dot_general(wot_v[DN:, h * gw:(h + 1) * gw], oh(h), _NT,
                                        preferred_element_type=f32)
                    yt = y if yt is None else yt + y
                return yt

            def npart():
                yn = None
                for h in range(Hkv):
                    y = lax.dot_general(oh(h), wot_v[:DN, h * gw:(h + 1) * gw], _NT,
                                        preferred_element_type=f32)
                    yn = y if yn is None else yn + y
                return yn

            if tt == 0:
                yn = npart()
                yt = tpart()
            else:
                yt = tpart()
                yn = npart()
            out_v[rows, :] = jnp.concatenate([yn, yt.T], axis=1).astype(out_v.dtype)
            out_copy(t).start()
        return carry

    @pl.when(step == 0)
    def _():
        phase0()
        lax.fori_loop(0, G, main, 0)

    @pl.when(step == 1)
    def _():
        wo_copy.wait()
        lax.fori_loop(0, NT2 // _P2T, oloop, 0)
        for t in range(NT2):
            out_copy(t).wait()


@jax.jit
def pallas_standalone__gqa_block_cached__near_ridge_kernel(
    x: jax.Array,
    k_cache: jax.Array,
    v_cache: jax.Array,
    wq: jax.Array,
    wo: jax.Array,
):
    B, Sq, D = x.shape
    _, Hkv, Sk, Dh = k_cache.shape
    M = B * Sq
    gw = 2 * Dh
    assert wq.shape[1] == Hkv * gw and Hkv % 2 == 0 and Hkv >= 6 and D % 128 != 0
    assert M % (128 * _P2T) == 0 and (B * Hkv - 1) % _U == 0 and Sq % _RC == 0
    assert Dh == 256 and Sk % _PG == 0 and _X0 < _X1 < M
    kern = functools.partial(_kernel, B=B, Sq=Sq, Hkv=Hkv, dh=Dh, scale=Dh ** -0.5)
    bf = jnp.bfloat16
    out = pl.pallas_call(
        kern,
        grid=(2,),
        in_specs=[pl.BlockSpec(memory_space=pl.ANY)] * 5,
        out_specs=pl.BlockSpec(memory_space=pl.ANY),
        out_shape=jax.ShapeDtypeStruct((M, D), x.dtype),
        scratch_shapes=[
            pltpu.VMEM((M, D), bf),
            pltpu.VMEM((Hkv, D, gw), bf),
            pltpu.VMEM((D, Hkv * gw), bf),
            pltpu.VMEM((Hkv, B, 2, Sq, Dh), bf),
            pltpu.VMEM((Hkv, 2, M, Dh), bf),
            pltpu.VMEM((_NBLK, _U, Sk, Dh), bf),
            pltpu.VMEM((_NBLK, _U, Sk, Dh), bf),
            pltpu.VMEM((Sk, Dh), bf),
            pltpu.VMEM((Sk, Dh), bf),
            pltpu.VMEM((M, D), bf),
            pltpu.SemaphoreType.DMA((11 + 2 * _NBLK,)),
            pltpu.SemaphoreType.DMA((M // 128,)),
        ],
        compiler_params=pltpu.CompilerParams(
            dimension_semantics=("arbitrary",),
            vmem_limit_bytes=100 * 1024 * 1024,
            disable_bounds_checks=True,
            disable_semaphore_checks=True,
        ),
    )(x.reshape(M, D), k_cache.reshape(B * Hkv, Sk, Dh), v_cache.reshape(B * Hkv, Sk, Dh),
      wq, wo.T)
    return out.reshape(B, Sq, D)
```

```python
import functools

import jax
import jax.numpy as jnp
from jax import lax
import jax.experimental.pallas as pl
import jax.experimental.pallas.tpu as pltpu

_LOG2E = 1.4426950408889634
_NT = (((1,), (1,)), ((), ()))
_RC = 16
_U = 7
_NBLK = 2
_KG = 256
_PG = 512
_PW = 2
_Q0 = 27
_S0 = 36
_P2T = 3
_X0 = 384
_X1 = 640


def _kernel(x_hbm, k_hbm, v_hbm, wq_hbm, wot_hbm, out_hbm,
            x_v, wq_v, wot_v, q_v, o_v, k_v, v_v, k0_v, vl_v, pc_v, lc_v, out_v,
            sem, sem_out,
            *, B, Sq, Hkv, dh, scale):
    G = (B * Hkv - 1) // _U
    sk = k_v.shape[-2]
    nt = sk // 128
    npart = nt // _PW
    gw = 2 * dh
    M = B * Sq
    NT2 = M // 128
    QL = (Hkv - 2) // 2
    DN = (out_v.shape[1] // 128) * 128
    step = pl.program_id(0)
    f32, bf16, u32 = jnp.float32, jnp.bfloat16, jnp.uint32
    escale = scale * _LOG2E

    def x_copy(i):
        lo, hi = ((0, _X0), (_X0, _X1), (_X1, M))[i]
        rows = pl.ds(lo, hi - lo)
        return pltpu.make_async_copy(x_hbm.at[rows], x_v.at[rows], sem.at[i])

    def wq0_copy(r):
        cols = pl.ds(r * dh, dh)
        return pltpu.make_async_copy(wq_hbm.at[:, cols], wq_v.at[0, :, cols], sem.at[3 + r])

    def wq_copy(j):
        s = 5 if j == 1 else 6 + (j - 2) // QL
        return pltpu.make_async_copy(
            wq_hbm.at[:, pl.ds(j * gw, gw)], wq_v.at[j], sem.at[s])

    k0_copy = pltpu.make_async_copy(k_hbm.at[0], k0_v, sem.at[8])
    vl_copy = pltpu.make_async_copy(v_hbm.at[B * Hkv - 1], vl_v, sem.at[9])
    wo_copy = pltpu.make_async_copy(wot_hbm, wot_v, sem.at[10])

    def kv_copies(g):
        slot = g % _NBLK if isinstance(g, int) else lax.rem(g, _NBLK)
        return (
            pltpu.make_async_copy(
                k_hbm.at[pl.ds(1 + g * _U, _U)], k_v.at[slot], sem.at[11 + slot]),
            pltpu.make_async_copy(
                v_hbm.at[pl.ds(g * _U, _U)], v_v.at[slot], sem.at[11 + _NBLK + slot]),
        )

    def out_rows(t):
        r0 = t * 128 if isinstance(t, int) else pl.multiple_of(t * 128, 128)
        return pl.ds(r0, 128)

    def out_copy(t):
        rows = out_rows(t)
        return pltpu.make_async_copy(out_v.at[rows], out_hbm.at[rows], sem_out.at[t])

    def store_q(q, r0, r1, j, heads):
        for b in range(B):
            lo, hi = max(r0, b * Sq), min(r1, (b + 1) * Sq)
            if lo < hi:
                for n, r in enumerate(heads):
                    q_v[j, b, r, lo - b * Sq:hi - b * Sq, :] = (
                        q[lo - r0:hi - r0, n * dh:(n + 1) * dh])

    def qproj(r0, r1, j, heads=(0, 1)):
        w = wq_v[j] if len(heads) == 2 else wq_v[j, :, heads[0] * dh:(heads[0] + 1) * dh]
        q = jnp.dot(x_v[r0:r1, :], w, preferred_element_type=f32).astype(bf16)
        store_q(q, r0, r1, j, heads)

    def tile(a, c, lo):
        return a[c * _RC:(c + 1) * _RC, lo:lo + 128]

    def rowmax(s, c, never, deps):
        mm = tile(s, c, (nt - 1) * 128)
        for t in range(nt - 1):
            mm = jnp.maximum(mm, tile(s, c, t * 128))
        if deps is not None:
            for t in range(deps.shape[1] // 128):
                mm = jnp.where(never, tile(deps, c, t * 128), mm)
        m = jnp.max(mm.astype(bf16).astype(f32), axis=-1, keepdims=True)
        return jnp.broadcast_to(m, (_RC, 128))

    def tie(blk, never, lp):
        return jnp.where(never, pltpu.bitcast(lp[:8] + lp[8:], u32), blk)

    def normalize(o, lps, never):
        lp = jnp.where(never, o[:, :128], jnp.concatenate(lps, axis=0))
        l = jnp.sum(lp, axis=-1, keepdims=True)
        r = pl.reciprocal(l, approx=True)
        r = r * (2.0 - l * r)
        return o * r

    def qloop(t, carry):
        never = t < 0
        grp = wq_v.at[pl.ds(2 + t * QL, QL)]
        pltpu.make_async_copy(grp, grp, sem.at[6 + t]).wait()
        q = q_v[0, 0, t]
        qproj(0, M, 2 + t * QL)
        s = lax.dot_general(q, k0_v[...], _NT, preferred_element_type=f32)
        nx = Sq // _RC
        ms = [rowmax(s, c, never, None) for c in range(nx)]
        lps = [None] * nx

        def portion(n, anchor):
            c, part = n // npart, n % npart
            m = jnp.where(never, anchor, ms[c])
            cols = slice(part * _PW * 128, (part + 1) * _PW * 128)
            sr = s[c * _RC:(c + 1) * _RC, cols].astype(bf16).astype(f32)
            p = jnp.exp2((sr - jnp.concatenate([m] * _PW, axis=1)) * escale)
            for tt in range(_PW):
                pt = p[:, tt * 128:(tt + 1) * 128]
                lps[c] = pt if lps[c] is None else lps[c] + pt
            pc_v[t, c * _RC:(c + 1) * _RC, cols] = p.astype(bf16)
            if part == npart - 1:
                lc_v[t, c * _RC:(c + 1) * _RC, :] = lps[c]
            return lps[c]

        j2 = 3 + t * QL
        nn_tiles = gw // 128
        nport = nx * npart
        prevq = None
        done = 0
        for b in range(B):
            x = x_v[b * Sq:(b + 1) * Sq, :]
            todo = (nport * b) // (B - 1) - done
            if todo:
                xa = pltpu.bitcast(x[:, :128], u32)
                vers = [[xa[c * 8:(c + 1) * 8] for c in range(nx)] for _ in range(nn_tiles)]
                for n in range(todo):
                    sl = n * (nn_tiles * nx) // todo
                    nn, c = sl // nx, sl % nx
                    lp = portion(done + n, tile(prevq, c, nn * 128))
                    vers[nn][c] = tie(vers[nn][c], never, lp)
                done += todo
                cols = []
                for nn in range(nn_tiles):
                    xt = jnp.concatenate(
                        [pltpu.bitcast(jnp.concatenate(vers[nn], axis=0), bf16), x[:, 128:]],
                        axis=1)
                    cols.append(jnp.dot(xt, wq_v[j2, :, nn * 128:(nn + 1) * 128],
                                        preferred_element_type=f32))
                qf = jnp.concatenate(cols, axis=1)
            else:
                qf = jnp.dot(x, wq_v[j2], preferred_element_type=f32)
            prevq = qf
            store_q(qf.astype(bf16), b * Sq, (b + 1) * Sq, j2, (0, 1))
        for j in range(2, QL):
            qproj(0, M, 2 + j + t * QL)
        return carry

    def phase0():
        x_copy(0).start()
        wq0_copy(0).start()
        wq0_copy(1).start()
        x_copy(1).start()
        x_copy(2).start()
        for j in range(1, 2 + QL):
            wq_copy(j).start()
        k0_copy.start()
        for j in range(2 + QL, Hkv):
            wq_copy(j).start()
        for g in range(_NBLK):
            for cp in kv_copies(g):
                cp.start()
        x_copy(0).wait()
        wq0_copy(0).wait()
        qproj(0, _X0, 0, (0,))
        wq0_copy(1).wait()
        x_copy(1).wait()
        qproj(0, _X0, 0, (1,))
        qproj(_X0, _X1, 0)
        x_copy(2).wait()
        wq_copy(1).wait()
        qproj(_X1, M, 0)
        qproj(0, M, 1)
        k0_copy.wait()
        lax.fori_loop(0, 2, qloop, 0)

    def main(g, carry):
        slot = lax.rem(g, _NBLK)
        never = g < 0
        for cp in kv_copies(g):
            cp.wait()
        us = [1 + g * _U + i for i in range(_U)]
        bs = [lax.div(u, Hkv) for u in us]
        hs = [lax.rem(u, Hkv) for u in us]
        nc = 2 * Sq // _RC
        nport = nc * npart
        ss = [None] * _U
        os_ = [None] * _U
        ons = [None] * _U
        ms = [None] * _U
        pp = [[[] for _ in range(nc)] for _ in range(_U)]
        lps = [[None] * nc for _ in range(_U)]

        def sm_max(i, deps):
            ms[i] = [rowmax(ss[i], c, never, deps) for c in range(nc)]

        def sm_portion(i, j, anchor):
            c, part = j // npart, j % npart
            m = jnp.where(never, anchor, ms[i][c])
            sc = ss[i][c * _RC:(c + 1) * _RC, part * _PW * 128:(part + 1) * _PW * 128]
            sr = sc.astype(bf16).astype(f32)
            for t in range(_PW):
                p = jnp.exp2((sr[:, t * 128:(t + 1) * 128] - m) * escale)
                pp[i][c].append(p)
                lps[i][c] = p if lps[i][c] is None else lps[i][c] + p
            return lps[i][c]

        def assign_slots(first, nslots):
            a = {}
            for j in range(nport):
                a.setdefault(first + j * (nslots - first) // nport, []).append(j)
            return a

        def qk(i):
            q = jnp.concatenate([q_v[hs[i], bs[i], 0], q_v[hs[i], bs[i], 1]], axis=0)
            k = k_v[slot, i]
            if i == 0:
                ss[i] = lax.dot_general(q, k, _NT, preferred_element_type=f32)
                return
            ng = sk // _KG
            assign = assign_slots(_Q0 if i == 1 else 0, ng * nc)
            qa = pltpu.bitcast(q[:, :128], u32)
            parts = []
            for t in range(ng):
                blks = []
                for c in range(nc):
                    blk = qa[c * 8:(c + 1) * 8]
                    for j in assign.get(t * nc + c, []):
                        anchor = tile(parts[t - 1], c, 0) if t else tile(os_[i - 2], c, 128)
                        blk = tie(blk, never, sm_portion(i - 1, j, anchor))
                    blks.append(blk)
                qt = jnp.concatenate(
                    [pltpu.bitcast(jnp.concatenate(blks, axis=0), bf16), q[:, 128:]], axis=1)
                parts.append(lax.dot_general(
                    qt, k[t * _KG:(t + 1) * _KG], _NT, preferred_element_type=f32))
            ss[i] = jnp.concatenate(parts, axis=1)

        def pv(i):
            v = v_v[slot, i + 1]
            if i != _U - 2:
                pb = jnp.concatenate(
                    [jnp.concatenate(r, axis=1) for r in pp[i]], axis=0).astype(bf16)
                return jnp.dot(pb, v, preferred_element_type=f32)
            ng = sk // _PG
            tg = _PG // 128
            assign = assign_slots(_S0, (dh // 128) * ng * nc)
            outs = []
            prev = None
            for half in range(dh // 128):
                acc = None
                for kg in range(ng):
                    rows = []
                    for c in range(nc):
                        tl = pp[i][c][kg * tg:(kg + 1) * tg]
                        blk = tl[0]
                        for j in assign.get((half * ng + kg) * nc + c, []):
                            lp = sm_portion(i + 1, j, tile(prev, c, 0))
                            blk = jnp.where(never, lp, blk)
                        rows.append(jnp.concatenate([blk] + tl[1:], axis=1))
                    pb = jnp.concatenate(rows, axis=0).astype(bf16)
                    y = jnp.dot(pb, v[kg * _PG:(kg + 1) * _PG, half * 128:(half + 1) * 128],
                                preferred_element_type=f32)
                    acc = y if acc is None else acc + y
                    prev = acc
                outs.append(acc)
            return jnp.concatenate(outs, axis=1)

        def store_o(on, b, h):
            ob = on.astype(bf16)
            rows = pl.ds(pl.multiple_of(b * Sq, 16), Sq)
            o_v[h, 0, rows, :] = ob[:Sq]
            o_v[h, 1, rows, :] = ob[Sq:]

        pc = jnp.concatenate([pc_v[0], pc_v[1]], axis=0)
        oc = jnp.dot(pc, v_v[slot, 0], preferred_element_type=f32)
        onc = normalize(oc, [lc_v[0], lc_v[1]], never)
        store_o(onc, lax.div(g * _U, Hkv), lax.rem(g * _U, Hkv))

        qk(0)
        for i in range(_U - 1):
            sm_max(i, ons[i - 2] if i >= 2 else (onc if i == 1 else None))
            qk(i + 1)
            if i == _U - 2:
                sm_max(i + 1, None)
            o = pv(i)
            on = normalize(o, lps[i], never)
            store_o(on, bs[i], hs[i])
            os_[i] = o
            ons[i] = on
        hc = nc // 2
        for c in range(nc):
            rr = slice((c % hc) * _RC, (c % hc + 1) * _RC)
            pc_v[c // hc, rr, :] = jnp.concatenate(pp[_U - 1][c], axis=1).astype(bf16)
            lc_v[c // hc, rr, :] = lps[_U - 1][c]

        @pl.when(g + _NBLK < G)
        def _():
            for cp in kv_copies(g + _NBLK):
                cp.start()

        @pl.when(g == G - _NBLK)
        def _():
            vl_copy.start()
            wo_copy.start()

        return carry

    def oloop(j, carry):
        never = j < 0
        r3n = Sq // (NT2 // _P2T)
        r3 = pl.ds(pl.multiple_of(j * r3n, 16), r3n)
        pc = jnp.concatenate([pc_v[0, r3, :], pc_v[1, r3, :]], axis=0)
        oc = jnp.dot(pc, vl_v[...], preferred_element_type=f32)
        on = normalize(oc, [lc_v[0, r3, :], lc_v[1, r3, :]], never)
        yt = None
        for tt in range(_P2T):
            t = j * _P2T + tt
            rows = out_rows(t)
            if tt == _P2T - 1:
                anchor = jnp.tile(yt[-8:, :], (2 * r3n // 8, dh // 128))
                ob = jnp.where(never, anchor, on).astype(bf16)
                ro = pl.ds(pl.multiple_of((B - 1) * Sq + j * r3n, 16), r3n)
                o_v[Hkv - 1, 0, ro, :] = ob[:r3n]
                o_v[Hkv - 1, 1, ro, :] = ob[r3n:]

            def oh(h):
                return jnp.concatenate([o_v[h, 0, rows, :], o_v[h, 1, rows, :]], axis=1)

            def tpart():
                acc = None
                for h in range(Hkv):
                    y = lax.dot_general(wot_v[DN:, h * gw:(h + 1) * gw], oh(h), _NT,
                                        preferred_element_type=f32)
                    acc = y if acc is None else acc + y
                return acc

            def npart_():
                acc = None
                for h in range(Hkv):
                    y = lax.dot_general(oh(h), wot_v[:DN, h * gw:(h + 1) * gw], _NT,
                                        preferred_element_type=f32)
                    acc = y if acc is None else acc + y
                return acc

            if tt == 0:
                yn = npart_()
                yt = tpart()
            else:
                yt = tpart()
                yn = npart_()
            out_v[rows, :] = jnp.concatenate([yn, yt.T], axis=1).astype(out_v.dtype)
            out_copy(t).start()
        return carry

    @pl.when(step == 0)
    def _():
        phase0()
        lax.fori_loop(0, G, main, 0)

    @pl.when(step == 1)
    def _():
        vl_copy.wait()
        wo_copy.wait()
        lax.fori_loop(0, NT2 // _P2T, oloop, 0)
        for t in range(NT2):
            out_copy(t).wait()


@jax.jit
def pallas_standalone__gqa_block_cached__near_ridge_kernel(
    x: jax.Array,
    k_cache: jax.Array,
    v_cache: jax.Array,
    wq: jax.Array,
    wo: jax.Array,
):
    B, Sq, D = x.shape
    _, Hkv, Sk, Dh = k_cache.shape
    M = B * Sq
    gw = 2 * Dh
    n2 = M // (128 * _P2T)
    assert wq.shape[1] == Hkv * gw and Hkv % 2 == 0 and Hkv >= 6 and D % 128 != 0
    assert M % (128 * _P2T) == 0 and (B * Hkv - 1) % _U == 0 and Sq % (_RC * n2) == 0
    assert Dh == 256 and Sk % _PG == 0 and _X0 < _X1 < M
    assert Sq // n2 <= 128 and M - 128 * _P2T <= (B - 1) * Sq
    kern = functools.partial(_kernel, B=B, Sq=Sq, Hkv=Hkv, dh=Dh, scale=Dh ** -0.5)
    bf = jnp.bfloat16
    out = pl.pallas_call(
        kern,
        grid=(2,),
        in_specs=[pl.BlockSpec(memory_space=pl.ANY)] * 5,
        out_specs=pl.BlockSpec(memory_space=pl.ANY),
        out_shape=jax.ShapeDtypeStruct((M, D), x.dtype),
        scratch_shapes=[
            pltpu.VMEM((M, D), bf),
            pltpu.VMEM((Hkv, D, gw), bf),
            pltpu.VMEM((D, Hkv * gw), bf),
            pltpu.VMEM((Hkv, B, 2, Sq, Dh), bf),
            pltpu.VMEM((Hkv, 2, M, Dh), bf),
            pltpu.VMEM((_NBLK, _U, Sk, Dh), bf),
            pltpu.VMEM((_NBLK, _U, Sk, Dh), bf),
            pltpu.VMEM((Sk, Dh), bf),
            pltpu.VMEM((Sk, Dh), bf),
            pltpu.VMEM((2, Sq, Sk), bf),
            pltpu.VMEM((2, Sq, 128), jnp.float32),
            pltpu.VMEM((M, D), bf),
            pltpu.SemaphoreType.DMA((11 + 2 * _NBLK,)),
            pltpu.SemaphoreType.DMA((M // 128,)),
        ],
        compiler_params=pltpu.CompilerParams(
            dimension_semantics=("arbitrary",),
            vmem_limit_bytes=100 * 1024 * 1024,
            disable_bounds_checks=True,
            disable_semaphore_checks=True,
        ),
    )(x.reshape(M, D), k_cache.reshape(B * Hkv, Sk, Dh), v_cache.reshape(B * Hkv, Sk, Dh),
      wq, wo.T)
    return out.reshape(B, Sq, D)
```

```python
import functools

import jax
import jax.numpy as jnp
from jax import lax
import jax.experimental.pallas as pl
import jax.experimental.pallas.tpu as pltpu

_LOG2E = 1.4426950408889634
_NT = (((1,), (1,)), ((), ()))
_RC = 16
_U = 7
_NBLK = 2
_KG = 256
_PG = 512
_PW = 2
_Q0 = 27
_S0 = 36
_P2T = 3
_X0 = 384
_X1 = 640


def _kernel(x_hbm, k_hbm, v_hbm, wq_hbm, wot_hbm, out_hbm,
            x_v, wq_v, wot_v, q_v, o_v, k_v, v_v, k0_v, vl_v, pc_v, lc_v, out_v,
            sem, sem_out,
            *, B, Sq, Hkv, dh, scale):
    G = (B * Hkv - 1) // _U
    sk = k_v.shape[-2]
    nt = sk // 128
    npart = nt // _PW
    gw = 2 * dh
    M = B * Sq
    NT2 = M // 128
    QL = (Hkv - 2) // 2
    DN = (out_v.shape[1] // 128) * 128
    step = pl.program_id(0)
    f32, bf16, u32 = jnp.float32, jnp.bfloat16, jnp.uint32
    escale = scale * _LOG2E

    def x_copy(i):
        lo, hi = ((0, _X0), (_X0, _X1), (_X1, M))[i]
        rows = pl.ds(lo, hi - lo)
        return pltpu.make_async_copy(x_hbm.at[rows], x_v.at[rows], sem.at[i])

    def wq0_copy(r):
        cols = pl.ds(r * dh, dh)
        return pltpu.make_async_copy(wq_hbm.at[:, cols], wq_v.at[0, :, cols], sem.at[3 + r])

    def wq_copy(j):
        s = 5 if j == 1 else 6 + (j - 2) // QL
        return pltpu.make_async_copy(
            wq_hbm.at[:, pl.ds(j * gw, gw)], wq_v.at[j], sem.at[s])

    k0_copy = pltpu.make_async_copy(k_hbm.at[0], k0_v, sem.at[8])
    vl_copy = pltpu.make_async_copy(v_hbm.at[B * Hkv - 1], vl_v, sem.at[9])
    wo_copy = pltpu.make_async_copy(wot_hbm, wot_v, sem.at[10])

    def kv_copies(g):
        slot = g % _NBLK if isinstance(g, int) else lax.rem(g, _NBLK)
        return (
            pltpu.make_async_copy(
                k_hbm.at[pl.ds(1 + g * _U, _U)], k_v.at[slot], sem.at[11 + slot]),
            pltpu.make_async_copy(
                v_hbm.at[pl.ds(g * _U, _U)], v_v.at[slot], sem.at[11 + _NBLK + slot]),
        )

    def out_rows(t):
        r0 = t * 128 if isinstance(t, int) else pl.multiple_of(t * 128, 128)
        return pl.ds(r0, 128)

    def out_copy(t):
        rows = out_rows(t)
        return pltpu.make_async_copy(out_v.at[rows], out_hbm.at[rows], sem_out.at[t])

    def store_q(q, r0, r1, j, heads):
        for b in range(B):
            lo, hi = max(r0, b * Sq), min(r1, (b + 1) * Sq)
            if lo < hi:
                for n, r in enumerate(heads):
                    q_v[j, b, r, lo - b * Sq:hi - b * Sq, :] = (
                        q[lo - r0:hi - r0, n * dh:(n + 1) * dh])

    def qproj(r0, r1, j, heads=(0, 1)):
        w = wq_v[j] if len(heads) == 2 else wq_v[j, :, heads[0] * dh:(heads[0] + 1) * dh]
        q = jnp.dot(x_v[r0:r1, :], w, preferred_element_type=f32).astype(bf16)
        store_q(q, r0, r1, j, heads)

    def tile(a, c, lo):
        return a[c * _RC:(c + 1) * _RC, lo:lo + 128]

    def rowmax(s, never, deps):
        mm = s[:, (nt - 1) * 128:]
        for t in range(nt - 1):
            mm = jnp.maximum(mm, s[:, t * 128:(t + 1) * 128])
        if deps is not None:
            for t in range(deps.shape[1] // 128):
                mm = lax.select(never, deps[:, t * 128:(t + 1) * 128], mm)
        m = jnp.max(mm.astype(bf16).astype(f32), axis=-1, keepdims=True)
        m = jnp.broadcast_to(m, mm.shape)
        return [tile(m, c, 0) for c in range(s.shape[0] // _RC)]

    def expo(sr, c, part, m):
        sc = sr[c * _RC:(c + 1) * _RC, part * _PW * 128:(part + 1) * _PW * 128]
        return jnp.exp2((sc - jnp.concatenate([m] * _PW, axis=1)) * escale)

    def tie(blk, never, lp):
        return lax.select(never, pltpu.bitcast(lp[:8] + lp[8:], u32), blk)

    def normalize(o, lps, never):
        lp = lax.select(never, o[:, :128], jnp.concatenate(lps, axis=0))
        l = jnp.sum(lp, axis=-1, keepdims=True)
        r = pl.reciprocal(l, approx=True)
        r = r * (2.0 - l * r)
        return o * r

    def qloop(t, carry):
        never = t < 0
        grp = wq_v.at[pl.ds(2 + t * QL, QL)]
        pltpu.make_async_copy(grp, grp, sem.at[6 + t]).wait()
        q = q_v[0, 0, t]
        qproj(0, M, 2 + t * QL)
        s = lax.dot_general(q, k0_v[...], _NT, preferred_element_type=f32)
        nx = Sq // _RC
        ms = rowmax(s, never, None)
        sr = s.astype(bf16).astype(f32)
        lps = [None] * nx

        def portion(n, anchor):
            c, part = n // npart, n % npart
            p = expo(sr, c, part, lax.select(never, anchor, ms[c]))
            cols = slice(part * _PW * 128, (part + 1) * _PW * 128)
            for tt in range(_PW):
                pt = p[:, tt * 128:(tt + 1) * 128]
                lps[c] = pt if lps[c] is None else lps[c] + pt
            pc_v[t, c * _RC:(c + 1) * _RC, cols] = p.astype(bf16)
            if part == npart - 1:
                lc_v[t, c * _RC:(c + 1) * _RC, :] = lps[c]
            return lps[c]

        j2 = 3 + t * QL
        nn_tiles = gw // 128
        nport = nx * npart
        prevq = None
        done = 0
        for b in range(B):
            x = x_v[b * Sq:(b + 1) * Sq, :]
            todo = (nport * b) // (B - 1) - done
            if todo:
                xa = pltpu.bitcast(x[:, :128], u32)
                vers = [[xa[c * 8:(c + 1) * 8] for c in range(nx)] for _ in range(nn_tiles)]
                for n in range(todo):
                    sl = n * (nn_tiles * nx) // todo
                    nn, c = sl // nx, sl % nx
                    lp = portion(done + n, tile(prevq, c, nn * 128))
                    vers[nn][c] = tie(vers[nn][c], never, lp)
                done += todo
                cols = []
                for nn in range(nn_tiles):
                    xt = jnp.concatenate(
                        [pltpu.bitcast(jnp.concatenate(vers[nn], axis=0), bf16), x[:, 128:]],
                        axis=1)
                    cols.append(jnp.dot(xt, wq_v[j2, :, nn * 128:(nn + 1) * 128],
                                        preferred_element_type=f32))
                qf = jnp.concatenate(cols, axis=1)
            else:
                qf = jnp.dot(x, wq_v[j2], preferred_element_type=f32)
            prevq = qf
            store_q(qf.astype(bf16), b * Sq, (b + 1) * Sq, j2, (0, 1))
        for j in range(2, QL):
            qproj(0, M, 2 + j + t * QL)
        return carry

    def phase0():
        x_copy(0).start()
        wq0_copy(0).start()
        wq0_copy(1).start()
        x_copy(1).start()
        x_copy(2).start()
        for j in range(1, 2 + QL):
            wq_copy(j).start()
        k0_copy.start()
        for j in range(2 + QL, Hkv):
            wq_copy(j).start()
        for g in range(_NBLK):
            for cp in kv_copies(g):
                cp.start()
        x_copy(0).wait()
        wq0_copy(0).wait()
        qproj(0, _X0, 0, (0,))
        wq0_copy(1).wait()
        x_copy(1).wait()
        qproj(0, _X0, 0, (1,))
        qproj(_X0, _X1, 0)
        x_copy(2).wait()
        wq_copy(1).wait()
        qproj(_X1, M, 0)
        qproj(0, M, 1)
        k0_copy.wait()
        lax.fori_loop(0, 2, qloop, 0)

    def main(g, carry):
        slot = lax.rem(g, _NBLK)
        never = g < 0
        for cp in kv_copies(g):
            cp.wait()
        us = [1 + g * _U + i for i in range(_U)]
        bs = [lax.div(u, Hkv) for u in us]
        hs = [lax.rem(u, Hkv) for u in us]
        nc = 2 * Sq // _RC
        nport = nc * npart
        ss = [None] * _U
        os_ = [None] * _U
        ons = [None] * _U
        ms = [None] * _U
        pp = [[[] for _ in range(nc)] for _ in range(_U)]
        lps = [[None] * nc for _ in range(_U)]

        def sm_max(i, deps):
            ms[i] = rowmax(ss[i], never, deps)
            ss[i] = ss[i].astype(bf16).astype(f32)

        def sm_portion(i, j, anchor):
            c, part = j // npart, j % npart
            p = expo(ss[i], c, part, lax.select(never, anchor, ms[i][c]))
            for t in range(_PW):
                pt = p[:, t * 128:(t + 1) * 128]
                pp[i][c].append(pt)
                lps[i][c] = pt if lps[i][c] is None else lps[i][c] + pt
            return lps[i][c]

        def assign_slots(first, nslots):
            a = {}
            for j in range(nport):
                a.setdefault(first + j * (nslots - first) // nport, []).append(j)
            return a

        def qk(i):
            q = jnp.concatenate([q_v[hs[i], bs[i], 0], q_v[hs[i], bs[i], 1]], axis=0)
            k = k_v[slot, i]
            if i == 0:
                ss[i] = lax.dot_general(q, k, _NT, preferred_element_type=f32)
                return
            ng = sk // _KG
            assign = assign_slots(_Q0 if i == 1 else 0, ng * nc)
            qa = pltpu.bitcast(q[:, :128], u32)
            qas = [qa[c * 8:(c + 1) * 8] for c in range(nc)]
            qb = q[:, 128:]
            parts = []
            for t in range(ng):
                blks = []
                for c in range(nc):
                    blk = qas[c]
                    for j in assign.get(t * nc + c, []):
                        anchor = tile(parts[t - 1], c, 0) if t else tile(os_[i - 2], c, 128)
                        blk = tie(blk, never, sm_portion(i - 1, j, anchor))
                    blks.append(blk)
                qt = jnp.concatenate(
                    [pltpu.bitcast(jnp.concatenate(blks, axis=0), bf16), qb], axis=1)
                parts.append(lax.dot_general(
                    qt, k[t * _KG:(t + 1) * _KG], _NT, preferred_element_type=f32))
            ss[i] = jnp.concatenate(parts, axis=1)

        def pv(i):
            v = v_v[slot, i + 1]
            if i != _U - 2:
                pb = jnp.concatenate(
                    [jnp.concatenate(r, axis=1) for r in pp[i]], axis=0).astype(bf16)
                return jnp.dot(pb, v, preferred_element_type=f32)
            ng = sk // _PG
            tg = _PG // 128
            assign = assign_slots(_S0, (dh // 128) * ng * nc)
            outs = []
            prev = None
            for half in range(dh // 128):
                acc = None
                for kg in range(ng):
                    rows = []
                    for c in range(nc):
                        tl = pp[i][c][kg * tg:(kg + 1) * tg]
                        blk = tl[0]
                        for j in assign.get((half * ng + kg) * nc + c, []):
                            lp = sm_portion(i + 1, j, tile(prev, c, 0))
                            blk = lax.select(never, lp, blk)
                        rows.append(jnp.concatenate([blk] + tl[1:], axis=1))
                    pb = jnp.concatenate(rows, axis=0).astype(bf16)
                    y = jnp.dot(pb, v[kg * _PG:(kg + 1) * _PG, half * 128:(half + 1) * 128],
                                preferred_element_type=f32)
                    acc = y if acc is None else acc + y
                    prev = acc
                outs.append(acc)
            return jnp.concatenate(outs, axis=1)

        def store_o(on, b, h):
            ob = on.astype(bf16)
            rows = pl.ds(pl.multiple_of(b * Sq, 16), Sq)
            o_v[h, 0, rows, :] = ob[:Sq]
            o_v[h, 1, rows, :] = ob[Sq:]

        pc = jnp.concatenate([pc_v[0], pc_v[1]], axis=0)
        oc = jnp.dot(pc, v_v[slot, 0], preferred_element_type=f32)
        onc = normalize(oc, [lc_v[0], lc_v[1]], never)
        store_o(onc, lax.div(g * _U, Hkv), lax.rem(g * _U, Hkv))

        qk(0)
        for i in range(_U - 1):
            sm_max(i, ons[i - 2] if i >= 2 else (onc if i == 1 else None))
            qk(i + 1)
            if i == _U - 2:
                sm_max(i + 1, None)
            o = pv(i)
            on = normalize(o, lps[i], never)
            store_o(on, bs[i], hs[i])
            os_[i] = o
            ons[i] = on
        hc = nc // 2
        for c in range(nc):
            rr = slice((c % hc) * _RC, (c % hc + 1) * _RC)
            pc_v[c // hc, rr, :] = jnp.concatenate(pp[_U - 1][c], axis=1).astype(bf16)
            lc_v[c // hc, rr, :] = lps[_U - 1][c]

        @pl.when(g + _NBLK < G)
        def _():
            for cp in kv_copies(g + _NBLK):
                cp.start()

        @pl.when(g == G - _NBLK)
        def _():
            vl_copy.start()
            wo_copy.start()

        return carry

    def oloop(j, carry):
        never = j < 0
        r3n = Sq // (NT2 // _P2T)
        r3 = pl.ds(pl.multiple_of(j * r3n, 16), r3n)
        pc = jnp.concatenate([pc_v[0, r3, :], pc_v[1, r3, :]], axis=0)
        oc = jnp.dot(pc, vl_v[...], preferred_element_type=f32)
        on = normalize(oc, [lc_v[0, r3, :], lc_v[1, r3, :]], never)
        yt = None
        for tt in range(_P2T):
            t = j * _P2T + tt
            rows = out_rows(t)
            if tt == _P2T - 1:
                anchor = jnp.concatenate([yt[-8:, :]] * (dh // 128), axis=1)
                anchor = jnp.concatenate([anchor] * (2 * r3n // 8), axis=0)
                ob = lax.select(never, anchor, on).astype(bf16)
                ro = pl.ds(pl.multiple_of((B - 1) * Sq + j * r3n, 16), r3n)
                o_v[Hkv - 1, 0, ro, :] = ob[:r3n]
                o_v[Hkv - 1, 1, ro, :] = ob[r3n:]

            def oh(h):
                return jnp.concatenate([o_v[h, 0, rows, :], o_v[h, 1, rows, :]], axis=1)

            def tpart():
                acc = None
                for h in range(Hkv):
                    y = lax.dot_general(wot_v[DN:, h * gw:(h + 1) * gw], oh(h), _NT,
                                        preferred_element_type=f32)
                    acc = y if acc is None else acc + y
                return acc

            def npart_():
                acc = None
                for h in range(Hkv):
                    y = lax.dot_general(oh(h), wot_v[:DN, h * gw:(h + 1) * gw], _NT,
                                        preferred_element_type=f32)
                    acc = y if acc is None else acc + y
                return acc

            if tt == 0:
                yn = npart_()
                yt = tpart()
            else:
                yt = tpart()
                yn = npart_()
            out_v[rows, :] = jnp.concatenate([yn, yt.T], axis=1).astype(out_v.dtype)
            out_copy(t).start()
        return carry

    @pl.when(step == 0)
    def _():
        phase0()
        lax.fori_loop(0, G, main, 0)

    @pl.when(step == 1)
    def _():
        vl_copy.wait()
        wo_copy.wait()
        lax.fori_loop(0, NT2 // _P2T, oloop, 0)
        for t in range(NT2):
            out_copy(t).wait()


@jax.jit
def pallas_standalone__gqa_block_cached__near_ridge_kernel(
    x: jax.Array,
    k_cache: jax.Array,
    v_cache: jax.Array,
    wq: jax.Array,
    wo: jax.Array,
):
    B, Sq, D = x.shape
    _, Hkv, Sk, Dh = k_cache.shape
    M = B * Sq
    gw = 2 * Dh
    n2 = M // (128 * _P2T)
    assert wq.shape[1] == Hkv * gw and Hkv % 2 == 0 and Hkv >= 6 and D % 128 != 0
    assert M % (128 * _P2T) == 0 and (B * Hkv - 1) % _U == 0 and Sq % (_RC * n2) == 0
    assert Dh == 256 and Sk % _PG == 0 and _X0 < _X1 < M
    assert Sq // n2 <= 128 and M - 128 * _P2T <= (B - 1) * Sq
    kern = functools.partial(_kernel, B=B, Sq=Sq, Hkv=Hkv, dh=Dh, scale=Dh ** -0.5)
    bf = jnp.bfloat16
    out = pl.pallas_call(
        kern,
        grid=(2,),
        in_specs=[pl.BlockSpec(memory_space=pl.ANY)] * 5,
        out_specs=pl.BlockSpec(memory_space=pl.ANY),
        out_shape=jax.ShapeDtypeStruct((M, D), x.dtype),
        scratch_shapes=[
            pltpu.VMEM((M, D), bf),
            pltpu.VMEM((Hkv, D, gw), bf),
            pltpu.VMEM((D, Hkv * gw), bf),
            pltpu.VMEM((Hkv, B, 2, Sq, Dh), bf),
            pltpu.VMEM((Hkv, 2, M, Dh), bf),
            pltpu.VMEM((_NBLK, _U, Sk, Dh), bf),
            pltpu.VMEM((_NBLK, _U, Sk, Dh), bf),
            pltpu.VMEM((Sk, Dh), bf),
            pltpu.VMEM((Sk, Dh), bf),
            pltpu.VMEM((2, Sq, Sk), bf),
            pltpu.VMEM((2, Sq, 128), jnp.float32),
            pltpu.VMEM((M, D), bf),
            pltpu.SemaphoreType.DMA((11 + 2 * _NBLK,)),
            pltpu.SemaphoreType.DMA((M // 128,)),
        ],
        compiler_params=pltpu.CompilerParams(
            dimension_semantics=("arbitrary",),
            vmem_limit_bytes=100 * 1024 * 1024,
            disable_bounds_checks=True,
            disable_semaphore_checks=True,
        ),
    )(x.reshape(M, D), k_cache.reshape(B * Hkv, Sk, Dh), v_cache.reshape(B * Hkv, Sk, Dh),
      wq, wo.T)
    return out.reshape(B, Sq, D)
```
